```python
import os as _os
_os.environ.setdefault("JAX_PLATFORMS", "cpu")
import jax
import jax.numpy as jnp

def _softmax(x, axis=-1):
    return jax.nn.softmax(x, axis=axis)
def _gelu(x):
    return jax.nn.gelu(x, approximate=True)
def _silu(x):
    return jax.nn.silu(x)
def _sigmoid(x):
    return jax.nn.sigmoid(x)
def _layernorm(x, axis=-1, eps=1e-5):
    m = jnp.mean(x, axis=axis, keepdims=True)
    v = jnp.var(x, axis=axis, keepdims=True)
    return (x - m) / jnp.sqrt(v + eps)
def _scatter_add(tgt, idx, src, axis=0):
    return tgt.at[idx].add(src)
def _segment_sum(src, seg, n):
    return jax.ops.segment_sum(src, seg, n)
class _Rng:
    def __init__(self, key):
        self._k = key
    def _next(self):
        self._k, sub = jax.random.split(self._k)
        return sub
    def normal(self, shape):
        return jax.random.normal(self._next(), shape, dtype=jnp.bfloat16)
    def randint(self, lo, hi, shape):
        return jax.random.randint(self._next(), shape, lo, hi, dtype=jnp.int32)
    def uniform(self, shape, lo=0.0, hi=1.0):
        return jax.random.uniform(self._next(), shape, jnp.bfloat16, lo, hi)
    def permutation(self, n):
        return jax.random.permutation(self._next(), n)


kernel_name = 'standalone__sliding_block_cached__sampling'

def setup_inputs():
    _rng = _Rng(jax.random.key(int.from_bytes(__import__("os").urandom(4), "little")))
    _w = (lambda a: (lambda t: t.astype(jnp.bfloat16) if jnp.issubdtype(t.dtype, jnp.floating) else t)(jnp.asarray(a)))
    B, Sq, D = 8, 4, 640
    Hq, Hkv, Sk, Dh = 32, 32, 4096, 192
    assert Hq % Hkv == 0, (Hq, Hkv)
    return {
        "x": _w((lambda *s: _rng.normal(s) * 0.8)(B, Sq, D)),
        "k_cache": _w((lambda *s: _rng.normal(s) * 0.8)(B, Hkv, Sk, Dh)),
        "v_cache": _w((lambda *s: _rng.normal(s) * 0.05)(B, Hkv, Sk, Dh)),
        "wq": _w((lambda *s: _rng.normal(s) * 0.8)(D, Hq * Dh) * (D ** -0.5)),
        "wo": _w((lambda *s: _rng.normal(s) * 0.05)(Hq * Dh, D) * ((Hq * Dh) ** -0.5)),
    }

def reference(x, k_cache, v_cache, wq, wo):
    B, Sq, D = x.shape
    Hq, Dh = 32, 192
    Hkv, Sk = k_cache.shape[1], k_cache.shape[2]
    W = min(4096, max(256, Sk // 4))
    rep = Hq // Hkv
    q = (lambda x, *d: x.transpose(*d))((x @ wq).reshape(B, Sq, Hq, Dh), 0, 2, 1, 3)
    k = jnp.repeat(k_cache[:, :, Sk - W:, :], rep, axis=1)
    v = jnp.repeat(v_cache[:, :, Sk - W:, :], rep, axis=1)
    scores = jnp.einsum("bhqd,bhkd->bhqk", q, k) * (Dh ** -0.5)
    p = _softmax(scores, axis=-1)
    o = jnp.einsum("bhqk,bhkd->bhqd", p, v)
    return (lambda x, *d: x.transpose(*d))(o, 0, 2, 1, 3).reshape(B, Sq, Hq * Dh) @ wo
```

```python
import functools
import jax
import jax.numpy as jnp
import jax.experimental.pallas as pl
import jax.experimental.pallas.tpu as pltpu

HB = 2


def _kernel(x_ref, wq_ref, kt_ref, vt_ref, wo_ref, out_ref,
            x2_ref, qbd_ref, o_ref, acc_ref, *, B, Sq, Dh, scale):
    hp = pl.program_id(0)
    b = pl.program_id(1)
    R = HB * Sq
    C = HB * Dh

    @pl.when(jnp.logical_and(hp == 0, b == 0))
    def _():
        for bb in range(B):
            x2_ref[bb * Sq:(bb + 1) * Sq, :] = x_ref[bb].astype(jnp.float32)
        acc_ref[...] = jnp.zeros_like(acc_ref)

    @pl.when(b == 0)
    def _():
        q = jnp.dot(x2_ref[...].astype(jnp.bfloat16), wq_ref[...],
                    preferred_element_type=jnp.float32)
        q = q.astype(jnp.bfloat16).astype(jnp.float32) * scale
        col = jax.lax.broadcasted_iota(jnp.int32, (Sq, C), 1)
        for bb in range(B):
            qb = q[bb * Sq:(bb + 1) * Sq, :]
            for h in range(HB):
                m = jnp.logical_and(col >= h * Dh, col < (h + 1) * Dh)
                qbd_ref[bb, h * Sq:(h + 1) * Sq, :] = jnp.where(m, qb, 0.0)

    qbd = qbd_ref[b].astype(jnp.bfloat16)
    s = jnp.dot(qbd, kt_ref[0], preferred_element_type=jnp.float32)
    m = jnp.max(s, axis=-1, keepdims=True)
    p = jnp.exp(s - m)
    l = jnp.sum(p, axis=-1, keepdims=True)
    o = jax.lax.dot_general(p.astype(jnp.bfloat16), vt_ref[0],
                            (((1,), (1,)), ((), ())),
                            preferred_element_type=jnp.float32)
    o = o / l
    col = jax.lax.broadcasted_iota(jnp.int32, (Sq, C), 1)
    osel = o[0:Sq, :]
    for h in range(1, HB):
        osel = jnp.where(col >= h * Dh, o[h * Sq:(h + 1) * Sq, :], osel)
    o_ref[b] = osel

    @pl.when(b == B - 1)
    def _():
        oall = jnp.concatenate([o_ref[bb] for bb in range(B)], axis=0)
        acc_ref[...] += jnp.dot(oall.astype(jnp.bfloat16), wo_ref[...],
                                preferred_element_type=jnp.float32)

    @pl.when(jnp.logical_and(hp == pl.num_programs(0) - 1, b == B - 1))
    def _():
        for bb in range(B):
            out_ref[bb] = acc_ref[bb * Sq:(bb + 1) * Sq, :].astype(out_ref.dtype)


@jax.jit
def pallas_standalone__sliding_block_cached__sampling_kernel(x, k_cache, v_cache, wq, wo):
    B, Sq, D = x.shape
    Hq, Dh = 32, 192
    Hkv, Sk = k_cache.shape[1], k_cache.shape[2]
    W = min(4096, max(256, Sk // 4))
    assert Hq == Hkv and Sk % W == 0
    kt = jnp.swapaxes(k_cache, 2, 3).reshape(B, Hkv * Dh, Sk)
    vt = jnp.swapaxes(v_cache, 2, 3).reshape(B, Hkv * Dh, Sk)
    C = HB * Dh
    wblk = Sk // W - 1
    kern = functools.partial(_kernel, B=B, Sq=Sq, Dh=Dh, scale=Dh ** -0.5)
    return pl.pallas_call(
        kern,
        grid=(Hq // HB, B),
        in_specs=[
            pl.BlockSpec((B, Sq, D), lambda h, b: (0, 0, 0)),
            pl.BlockSpec((D, C), lambda h, b: (0, h)),
            pl.BlockSpec((1, C, W), lambda h, b: (b, h, wblk)),
            pl.BlockSpec((1, C, W), lambda h, b: (b, h, wblk)),
            pl.BlockSpec((C, D), lambda h, b: (h, 0)),
        ],
        out_specs=pl.BlockSpec((B, Sq, D), lambda h, b: (0, 0, 0)),
        out_shape=jax.ShapeDtypeStruct((B, Sq, D), x.dtype),
        scratch_shapes=[
            pltpu.VMEM((B * Sq, D), jnp.float32),
            pltpu.VMEM((B, HB * Sq, C), jnp.float32),
            pltpu.VMEM((B, Sq, C), jnp.float32),
            pltpu.VMEM((B * Sq, D), jnp.float32),
        ],
        compiler_params=pltpu.CompilerParams(
            dimension_semantics=("arbitrary", "arbitrary"),
            vmem_limit_bytes=64 * 1024 * 1024,
        ),
    )(x, wq, kt, vt, wo)
```

```python
import functools
import os
import jax
import jax.numpy as jnp
import jax.experimental.pallas as pl
import jax.experimental.pallas.tpu as pltpu

NBUF = int(os.environ.get("NBUF", "5"))
NG = int(os.environ.get("NG", "3"))
QROWS = 128
LAST = 128


def _wo_pieces(n_groups, C):
    pieces = [(g * C, C) for g in range(n_groups - 1)]
    base = (n_groups - 1) * C
    pieces += [(base + k * LAST, LAST) for k in range(C // LAST)]
    return pieces


def _kernel(x_hbm, wq_hbm, kt_hbm, vt_hbm, wo_hbm, out_ref,
            xbuf, wqbuf, wobuf, kvbuf, x2_ref, qacc_ref, zq_ref, o_ref,
            xsem, qsem, osem, kvsem, *, B, Sq, D, H, Dh, Sk, W, scale):
    C = 2 * Dh
    G = H // 2
    J = B // 2
    N = G * B
    R = 2 * Sq
    T = C // 16
    U = T // NG
    NQ = D // QROWS
    DIST = NBUF - 1
    pieces = _wo_pieces(G, C)
    NO = len(pieces)

    def x_copy():
        return pltpu.make_async_copy(x_hbm, xbuf, xsem.at[0])

    def wq_copy(p):
        rows = pl.ds(p * QROWS, QROWS)
        return pltpu.make_async_copy(wq_hbm.at[rows], wqbuf.at[rows], qsem.at[p])

    def wo_copy(p):
        rows = pl.ds(pieces[p][0], pieces[p][1])
        return pltpu.make_async_copy(wo_hbm.at[rows], wobuf.at[rows], osem.at[p])

    def kv_start(i, slot, u, par):
        for a, src in enumerate((kt_hbm, vt_hbm)):
            pltpu.make_async_copy(
                src.at[pl.ds(i * T + u * NG, NG), par, :, pl.ds(Sk - W, W)],
                kvbuf.at[slot, a, pl.ds(u * NG, NG), par],
                kvsem.at[slot]).start(priority=par)

    def kv_wait(slot):
        pltpu.make_async_copy(kvbuf.at[slot], kvbuf.at[slot], kvsem.at[slot]).wait()

    x_copy().start()
    for p in range(NQ):
        wq_copy(p).start()
    x_copy().wait()
    for b in range(B):
        x2_ref[b * Sq:(b + 1) * Sq, :] = xbuf[b].astype(jnp.float32)
    for p in range(NQ):
        wq_copy(p).wait()
        if p == NQ - 2:
            for u in range(U):
                kv_start(0, 0, u, 0)
                kv_start(0, 0, u, 1)
        xp = x2_ref[:, p * QROWS:(p + 1) * QROWS].astype(jnp.bfloat16)
        part = jnp.dot(xp, wqbuf[p * QROWS:(p + 1) * QROWS, :],
                       preferred_element_type=jnp.float32)
        if p == 0:
            qacc_ref[...] = part
        else:
            qacc_ref[...] += part

    row = jax.lax.broadcasted_iota(jnp.int32, (R, C), 0)
    col = jax.lax.broadcasted_iota(jnp.int32, (R, C), 1)
    first_head = col < Dh
    diag = (row < Sq) == first_head
    for g in range(G):
        for j in range(J):
            q = qacc_ref[j * R:(j + 1) * R, g * C:(g + 1) * C]
            q = q.astype(jnp.bfloat16).astype(jnp.float32)
            z = jnp.where(first_head, q, pltpu.roll(q, Sq, 0))
            zq_ref[2 * j, g] = jnp.where(diag, z, 0.0)
            zq_ref[2 * j + 1, g] = jnp.where(diag, 0.0, z)

    for i in range(1, DIST):
        for u in range(U):
            kv_start(i, i, u, 0)
            kv_start(i, i, u, 1)

    def body(i, carry):
        slot = i % NBUF
        nxt = i + DIST
        nslot = nxt % NBUF
        more = nxt < N
        nx = jnp.minimum(nxt, N - 1)

        def issue(u):
            @pl.when(more)
            def _():
                if u > 0:
                    kv_start(nx, nslot, u - 1, 1)
                if u < U:
                    kv_start(nx, nslot, u, 0)

        @pl.when(nxt == N)
        def _():
            for p in range(NO):
                wo_copy(p).start(priority=1)

        b = i // G
        g = i % G
        qbd = zq_ref[b, g].astype(jnp.bfloat16)
        kv_wait(slot)

        def tile(a, c0, cn, t0=0, tn=T):
            v = kvbuf[slot, a, t0:t0 + tn, :, :, c0:c0 + cn]
            return v.reshape(tn * 16, cn)

        half = W // 2
        issue(0)
        s0 = jnp.dot(qbd, tile(0, 0, half), preferred_element_type=jnp.float32)
        issue(1)
        s1 = jnp.dot(qbd, tile(0, half, half), preferred_element_type=jnp.float32)
        issue(2)
        s = jnp.concatenate([s0, s1], axis=1) * scale
        m = jnp.max(s, axis=-1, keepdims=True)
        p = jnp.exp(s - m)
        l = jnp.sum(p, axis=-1, keepdims=True)
        pb = p.astype(jnp.bfloat16)
        o = None
        q4 = W // 4
        for c in range(4):
            issue(3 + c)
            part = jax.lax.dot_general(pb[:, c * q4:(c + 1) * q4], tile(1, c * q4, q4),
                                       (((1,), (1,)), ((), ())),
                                       preferred_element_type=jnp.float32)
            o = part if o is None else o + part
        for u in range(7, U + 1):
            issue(u)
        o_ref[g, b] = o / l
        return carry

    jax.lax.fori_loop(0, N, body, 0)

    acc = None
    for p in range(NO):
        r0, rn = pieces[p]
        g, c0 = r0 // C, r0 % C
        blocks = []
        for j in range(J):
            zo = jnp.where(diag, o_ref[g, 2 * j], o_ref[g, 2 * j + 1])
            blocks.append(jnp.where(first_head, zo, pltpu.roll(zo, Sq, 0)))
        lhs = jnp.concatenate(blocks, axis=0)[:, c0:c0 + rn].astype(jnp.bfloat16)
        wo_copy(p).wait()
        part = jnp.dot(lhs, wobuf[r0:r0 + rn, :], preferred_element_type=jnp.float32)
        acc = part if acc is None else acc + part
    for b in range(B):
        out_ref[b] = acc[b * Sq:(b + 1) * Sq, :].astype(out_ref.dtype)


@jax.jit
def pallas_standalone__sliding_block_cached__sampling_kernel(x, k_cache, v_cache, wq, wo):
    B, Sq, D = x.shape
    Hq, Dh = 32, 192
    Hkv, Sk = k_cache.shape[1], k_cache.shape[2]
    W = min(4096, max(256, Sk // 4))
    assert Hq == Hkv
    kt = jnp.swapaxes(k_cache, 2, 3).reshape(B * Hkv * Dh // 16, 2, 8, Sk)
    vt = jnp.swapaxes(v_cache, 2, 3).reshape(B * Hkv * Dh // 16, 2, 8, Sk)
    C = 2 * Dh
    G, J, R = Hq // 2, B // 2, 2 * Sq
    n_wo = len(_wo_pieces(G, C))
    kern = functools.partial(_kernel, B=B, Sq=Sq, D=D, H=Hq, Dh=Dh, Sk=Sk, W=W,
                             scale=Dh ** -0.5)
    any_spec = pl.BlockSpec(memory_space=pl.ANY)
    return pl.pallas_call(
        kern,
        in_specs=[any_spec] * 5,
        out_specs=pl.BlockSpec((B, Sq, D), lambda: (0, 0, 0)),
        out_shape=jax.ShapeDtypeStruct((B, Sq, D), x.dtype),
        scratch_shapes=[
            pltpu.VMEM((B, Sq, D), x.dtype),
            pltpu.VMEM((D, Hq * Dh), wq.dtype),
            pltpu.VMEM((Hq * Dh, D), wo.dtype),
            pltpu.VMEM((NBUF, 2, C // 16, 2, 8, W), k_cache.dtype),
            pltpu.VMEM((B * Sq, D), jnp.float32),
            pltpu.VMEM((B * Sq, Hq * Dh), jnp.float32),
            pltpu.VMEM((B, G, R, C), jnp.float32),
            pltpu.VMEM((G, B, R, C), jnp.float32),
            pltpu.SemaphoreType.DMA((1,)),
            pltpu.SemaphoreType.DMA((D // QROWS,)),
            pltpu.SemaphoreType.DMA((n_wo,)),
            pltpu.SemaphoreType.DMA((NBUF,)),
        ],
        compiler_params=pltpu.CompilerParams(
            vmem_limit_bytes=64 * 1024 * 1024,
            disable_semaphore_checks=True,
        ),
    )(x, wq, kt, vt, wo)
```

```python
import dataclasses
import functools

import jax
import jax.numpy as jnp
import jax.experimental.pallas as pl
import jax.experimental.pallas.tpu as pltpu

DIST = 4
NG = 2
LAG = 16
WQC = 2048
WOC = 32
WOS = 16
UNIT = 128
PCH = 12
HI, LO = 0, 1


def _wo_plan(rows):
    small_rows = LAG * WOS
    half = (rows - small_rows) // 2
    assert small_rows % UNIT == 0 and half % UNIT == 0 and half % WOC == 0
    assert 2 * half + small_rows == rows and (PCH * WOC) % UNIT == 0
    nnorm = half // WOC
    return half, nnorm, pl.cdiv(nnorm, PCH), small_rows // UNIT


def _kernel(x_hbm, wq_hbm, kt_hbm, vt_hbm, wo_hbm, out_ref,
            xbuf, wqbuf, wobuf, kvbuf, x2_ref, zq_ref, o_ref, oall_ref,
            qsem, osem, kvsem, *, B, Sq, D, H, Dh, Sk, W, scale):
    C = 2 * Dh
    G = H // 2
    J = B // 2
    N = G * B
    R = 2 * Sq
    T = C // 16
    U = T // NG
    DPS = 2 * U
    NBUF = DIST + 1
    SHIFT = LAG // 2
    HALF, NNORM, NPIECE, NSU = _wo_plan(H * Dh)
    KQ = H * Dh // WQC
    NQ = (D // 16) * KQ
    assert pl.cdiv(SHIFT, U) < DIST

    def wq_start(m, par):
        row0 = par * (D // 2) + (m // KQ) * 8
        col0 = (m % KQ) * WQC
        if not isinstance(m, int):
            row0 = pl.multiple_of(row0, 8)
            col0 = pl.multiple_of(col0, WQC)
        idx = (pl.ds(row0, 8), pl.ds(col0, WQC))
        pltpu.make_async_copy(wq_hbm.at[idx], wqbuf.at[idx],
                              qsem.at[1]).start(priority=par)

    def kv_start(i, u, a, par):
        slot = i % NBUF
        pltpu.make_async_copy(
            (kt_hbm, vt_hbm)[a].at[pl.ds(i * T + u * NG, NG), par, :, pl.ds(Sk - W, W)],
            kvbuf.at[slot, a, pl.ds(u * NG, NG), par],
            kvsem.at[slot]).start(priority=par)

    def wo_start(m, par):
        if isinstance(m, int) and m >= NNORM:
            r0, rn = 2 * HALF + (m - NNORM) * WOS, WOS
            sem = osem.at[2 * NPIECE + (r0 - 2 * HALF) // UNIT]
        else:
            r0, rn = par * HALF + m * WOC, WOC
            sem = osem.at[par * NPIECE + m // PCH]
            if not isinstance(m, int):
                r0 = pl.multiple_of(r0, WOC)
        rows = pl.ds(r0, rn)
        pltpu.make_async_copy(wo_hbm.at[rows], wobuf.at[rows], sem).start(priority=par)

    def wait_all(ref, sem):
        pltpu.make_async_copy(ref, ref, sem).wait()

    def static_issue(d, par):
        if d < 0:
            wq_start(NQ + d, par)
        elif d < N * DPS:
            kv_start(d // DPS, (d % DPS) // 2, d % 2, par)
        elif d - N * DPS < NNORM + (LAG if par == LO else 0):
            wo_start(d - N * DPS, par)

    def q_issue(m, carry):
        wq_start(m, LO)

        @pl.when(m >= LAG)
        def _():
            wq_start(jnp.maximum(m - LAG, 0), HI)
        return carry

    jax.lax.fori_loop(0, NQ, q_issue, 0)
    x_copy = pltpu.make_async_copy(x_hbm, xbuf, qsem.at[0])
    x_copy.start(priority=HI)
    for d in range(DIST * DPS):
        static_issue(d, LO)
        static_issue(d - LAG, HI)

    x_copy.wait()
    for b in range(B):
        x2_ref[b * Sq:(b + 1) * Sq, :] = xbuf[b].astype(jnp.float32)
    wait_all(wqbuf, qsem.at[1])

    row = jax.lax.broadcasted_iota(jnp.int32, (R, C), 0)
    col = jax.lax.broadcasted_iota(jnp.int32, (R, C), 1)
    first_head = col < Dh
    diag = (row < Sq) == first_head

    def body(i, carry):
        slot = i % NBUF
        b = i // G
        g = i % G

        def dyn_issue(step, u, e, par):
            @pl.when(step < N)
            def _():
                kv_start(jnp.minimum(step, N - 1), u, e, par)

            m = (step - N) * DPS + 2 * u + e

            @pl.when(jnp.logical_and(m >= 0, m < NNORM))
            def _():
                wo_start(jnp.clip(m, 0, NNORM - 1), par)

        def issue(u):
            for e in range(2):
                dyn_issue(i + DIST, u, e, LO)
                dyn_issue(i + DIST + (u - SHIFT) // U, (u - SHIFT) % U, e, HI)

        @pl.when(i < G)
        def _():
            cols = pl.ds(pl.multiple_of(g * C, 128), C)
            q = jnp.dot(x2_ref[...].astype(jnp.bfloat16), wqbuf[:, cols],
                        preferred_element_type=jnp.float32)
            q = q.astype(jnp.bfloat16).astype(jnp.float32)
            for j in range(J):
                qj = q[j * R:(j + 1) * R, :]
                z = jnp.where(first_head, qj, pltpu.roll(qj, Sq, 0))
                zq_ref[2 * j, g] = jnp.where(diag, z, 0.0)
                zq_ref[2 * j + 1, g] = jnp.where(diag, 0.0, z)

        qbd = zq_ref[b, g].astype(jnp.bfloat16)
        wait_all(kvbuf.at[slot], kvsem.at[slot])

        def tile(a, c0, cn):
            return kvbuf[slot, a, :, :, :, c0:c0 + cn].reshape(C, cn)

        nqk = U // 3
        npv = U - nqk
        cw = W // nqk
        parts = []
        for c in range(nqk):
            issue(c)
            parts.append(jnp.dot(qbd, tile(0, c * cw, cw),
                                 preferred_element_type=jnp.float32))
        s = jnp.concatenate(parts, axis=1) * scale
        m = jnp.max(s, axis=-1, keepdims=True)
        p = jnp.exp(s - m)
        l = jnp.sum(p, axis=-1, keepdims=True)
        pb = p.astype(jnp.bfloat16)
        cw = W // npv
        o = None
        for c in range(npv):
            issue(nqk + c)
            part = jax.lax.dot_general(pb[:, c * cw:(c + 1) * cw], tile(1, c * cw, cw),
                                       (((1,), (1,)), ((), ())),
                                       preferred_element_type=jnp.float32)
            o = part if o is None else o + part
        o_ref[g, b] = o / l
        return carry

    jax.lax.fori_loop(0, N, body, 0)

    nxt = {LO: N * DPS + min(DIST * DPS, NNORM),
           HI: N * DPS + min(DIST * DPS - LAG, NNORM)}

    def issue_some(cnt):
        for _ in range(cnt):
            for par in (LO, HI):
                static_issue(nxt[par], par)
                nxt[par] += 1

    issue_some(8)
    for g in range(G):
        for j in range(J):
            zo = jnp.where(diag, o_ref[g, 2 * j], o_ref[g, 2 * j + 1])
            oall_ref[j * R:(j + 1) * R, g * C:(g + 1) * C] = jnp.where(
                first_head, zo, pltpu.roll(zo, Sq, 0))

    pieces = []
    for k in range(NPIECE):
        last = min((k + 1) * PCH, NNORM)
        for par in (HI, LO):
            pieces.append((par * NPIECE + k, par * HALF + k * PCH * WOC,
                           (last - k * PCH) * WOC, par, last))
    for k in range(NSU):
        pieces.append((2 * NPIECE + k, 2 * HALF + k * UNIT, UNIT, LO,
                       NNORM + (k + 1) * UNIT // WOS))
    acc = None
    for p, r0, rn, par, last in pieces:
        issue_some(6)
        assert nxt[par] >= N * DPS + last
        lhs = oall_ref[:, r0:r0 + rn].astype(jnp.bfloat16)
        wait_all(wobuf.at[pl.ds(r0, rn)], osem.at[p])
        part = jnp.dot(lhs, wobuf[r0:r0 + rn, :], preferred_element_type=jnp.float32)
        acc = part if acc is None else acc + part
    for b in range(B):
        out_ref[b] = acc[b * Sq:(b + 1) * Sq, :].astype(out_ref.dtype)


def _compiler_params():
    params = dict(vmem_limit_bytes=64 * 1024 * 1024)
    fields = {f.name for f in dataclasses.fields(pltpu.CompilerParams)}
    for name in ("disable_bounds_checks", "disable_semaphore_checks"):
        if name in fields:
            params[name] = True
    return pltpu.CompilerParams(**params)


@jax.jit
def pallas_standalone__sliding_block_cached__sampling_kernel(
    x: jax.Array,
    k_cache: jax.Array,
    v_cache: jax.Array,
    wq: jax.Array,
    wo: jax.Array,
):
    B, Sq, D = x.shape
    Hq, Dh = 32, 192
    Hkv, Sk = k_cache.shape[1], k_cache.shape[2]
    W = min(4096, max(256, Sk // 4))
    assert Hq == Hkv and B % 2 == 0 and 2 * Sq == 8 and (Sk - W) % 128 == 0
    kt = jnp.swapaxes(k_cache, 2, 3).reshape(B * Hkv * Dh // 16, 2, 8, Sk)
    vt = jnp.swapaxes(v_cache, 2, 3).reshape(B * Hkv * Dh // 16, 2, 8, Sk)
    C = 2 * Dh
    G, R = Hq // 2, 2 * Sq
    _, _, npiece, nsu = _wo_plan(Hq * Dh)
    kern = functools.partial(_kernel, B=B, Sq=Sq, D=D, H=Hq, Dh=Dh, Sk=Sk, W=W,
                             scale=Dh ** -0.5)
    return pl.pallas_call(
        kern,
        in_specs=[pl.BlockSpec(memory_space=pl.ANY)] * 5,
        out_specs=pl.BlockSpec((B, Sq, D), lambda: (0, 0, 0)),
        out_shape=jax.ShapeDtypeStruct((B, Sq, D), x.dtype),
        scratch_shapes=[
            pltpu.VMEM((B, Sq, D), x.dtype),
            pltpu.VMEM((D, Hq * Dh), wq.dtype),
            pltpu.VMEM((Hq * Dh, D), wo.dtype),
            pltpu.VMEM((DIST + 1, 2, C // 16, 2, 8, W), k_cache.dtype),
            pltpu.VMEM((B * Sq, D), jnp.float32),
            pltpu.VMEM((B, G, R, C), jnp.float32),
            pltpu.VMEM((G, B, R, C), jnp.float32),
            pltpu.VMEM((B * Sq, Hq * Dh), jnp.float32),
            pltpu.SemaphoreType.DMA((2,)),
            pltpu.SemaphoreType.DMA((2 * npiece + nsu,)),
            pltpu.SemaphoreType.DMA((DIST + 1,)),
        ],
        compiler_params=_compiler_params(),
    )(x, wq, kt, vt, wo)
```

```python
import dataclasses
import functools

import jax
import jax.numpy as jnp
import jax.experimental.pallas as pl
import jax.experimental.pallas.tpu as pltpu

DIST = 4
NG = 2
LAG = 16
WQC = 2048
WOC = 32
WOS = 16
UNIT = 128
PCH = 12
HI, LO = 0, 1


def _wo_plan(rows):
    small_rows = LAG * WOS
    half = (rows - small_rows) // 2
    assert small_rows % UNIT == 0 and half % UNIT == 0 and half % WOC == 0
    assert 2 * half + small_rows == rows and (PCH * WOC) % UNIT == 0
    nnorm = half // WOC
    return half, nnorm, pl.cdiv(nnorm, PCH), small_rows // UNIT


def _kernel(x_hbm, wq_hbm, kt_hbm, vt_hbm, wo_hbm, out_ref,
            xbuf, wqbuf, wobuf, kvbuf, x2_ref, zq_ref, o_ref, oall_ref,
            qsem, osem, kvsem, *, B, Sq, D, H, Dh, Sk, W, scale):
    C = 2 * Dh
    G = H // 2
    J = B // 2
    N = G * B
    R = 2 * Sq
    T = C // 16
    U = T // NG
    DPS = 2 * U
    NBUF = DIST + 1
    SHIFT = LAG // 2
    HALF, NNORM, NPIECE, NSU = _wo_plan(H * Dh)
    KQ = H * Dh // WQC
    NQ = (D // 16) * KQ
    assert pl.cdiv(SHIFT, U) < DIST and N - DIST >= G

    def wq_start(m, par):
        row0 = par * (D // 2) + (m // KQ) * 8
        col0 = (m % KQ) * WQC
        if not isinstance(m, int):
            row0 = pl.multiple_of(row0, 8)
            col0 = pl.multiple_of(col0, WQC)
        idx = (pl.ds(row0, 8), pl.ds(col0, WQC))
        pltpu.make_async_copy(wq_hbm.at[idx], wqbuf.at[idx],
                              qsem.at[1]).start(priority=par)

    def kv_start(i, u, a, par):
        slot = i % NBUF
        pltpu.make_async_copy(
            (kt_hbm, vt_hbm)[a].at[pl.ds(i * T + u * NG, NG), par, :, pl.ds(Sk - W, W)],
            kvbuf.at[slot, a, pl.ds(u * NG, NG), par],
            kvsem.at[slot]).start(priority=par)

    def wo_start(m, par):
        if m >= NNORM:
            r0, rn = 2 * HALF + (m - NNORM) * WOS, WOS
            sem = osem.at[2 * NPIECE + (r0 - 2 * HALF) // UNIT]
        else:
            r0, rn = par * HALF + m * WOC, WOC
            sem = osem.at[par * NPIECE + m // PCH]
        rows = pl.ds(r0, rn)
        pltpu.make_async_copy(wo_hbm.at[rows], wobuf.at[rows], sem).start(priority=par)

    def wait_all(ref, sem):
        pltpu.make_async_copy(ref, ref, sem).wait()

    def static_issue(d, par):
        if d < 0:
            wq_start(NQ + d, par)
        elif d < N * DPS:
            kv_start(d // DPS, (d % DPS) // 2, d % 2, par)
        elif d - N * DPS < NNORM + (LAG if par == LO else 0):
            wo_start(d - N * DPS, par)

    for m in range(LAG):
        wq_start(m, LO)

    def q_issue(m, carry):
        wq_start(m + LAG, LO)
        wq_start(m, HI)
        return carry

    jax.lax.fori_loop(0, NQ - LAG, q_issue, 0)
    x_copy = pltpu.make_async_copy(x_hbm, xbuf, qsem.at[0])
    x_copy.start(priority=HI)
    for d in range(DIST * DPS):
        static_issue(d, LO)
        static_issue(d - LAG, HI)

    x_copy.wait()
    for b in range(B):
        x2_ref[b * Sq:(b + 1) * Sq, :] = xbuf[b].astype(jnp.float32)
    wait_all(wqbuf, qsem.at[1])

    row = jax.lax.broadcasted_iota(jnp.int32, (R, C), 0)
    col = jax.lax.broadcasted_iota(jnp.int32, (R, C), 1)
    first_head = col < Dh
    diag = (row < Sq) == first_head

    def step(i, issue):
        slot = i % NBUF
        b = i // G
        g = i % G

        def q_project():
            cols = pl.ds(pl.multiple_of(g * C, 128), C)
            q = jnp.dot(x2_ref[...].astype(jnp.bfloat16), wqbuf[:, cols],
                        preferred_element_type=jnp.float32)
            q = q.astype(jnp.bfloat16).astype(jnp.float32)
            for j in range(J):
                qj = q[j * R:(j + 1) * R, :]
                z = jnp.where(first_head, qj, pltpu.roll(qj, Sq, 0))
                zq_ref[2 * j, g] = jnp.where(diag, z, 0.0)
                zq_ref[2 * j + 1, g] = jnp.where(diag, 0.0, z)

        if not isinstance(i, int):
            pl.when(i < G)(q_project)

        qbd = zq_ref[b, g].astype(jnp.bfloat16)
        wait_all(kvbuf.at[slot], kvsem.at[slot])

        def tile(a, c0, cn):
            return kvbuf[slot, a, :, :, :, c0:c0 + cn].reshape(C, cn)

        nqk = U // 3
        npv = U - nqk
        cw = W // nqk
        parts = []
        for c in range(nqk):
            issue(c)
            parts.append(jnp.dot(qbd, tile(0, c * cw, cw),
                                 preferred_element_type=jnp.float32))
        s = jnp.concatenate(parts, axis=1) * scale
        m = jnp.max(s, axis=-1, keepdims=True)
        p = jnp.exp(s - m)
        l = jnp.sum(p, axis=-1, keepdims=True)
        pb = p.astype(jnp.bfloat16)
        cw = W // npv
        o = None
        for c in range(npv):
            issue(nqk + c)
            part = jax.lax.dot_general(pb[:, c * cw:(c + 1) * cw], tile(1, c * cw, cw),
                                       (((1,), (1,)), ((), ())),
                                       preferred_element_type=jnp.float32)
            o = part if o is None else o + part
        o_ref[g, b] = o / l

    def body(i, carry):
        def issue(u):
            for e in range(2):
                kv_start(i + DIST, u, e, LO)
                kv_start(i + DIST + (u - SHIFT) // U, (u - SHIFT) % U, e, HI)

        step(i, issue)
        return carry

    jax.lax.fori_loop(0, N - DIST, body, 0)

    nxt = {LO: N * DPS, HI: N * DPS - LAG}

    def issue_some(cnt):
        for _ in range(cnt):
            for par in (LO, HI):
                static_issue(nxt[par], par)
                nxt[par] += 1

    for i in range(N - DIST, N):
        assert nxt[HI] >= (i + 1) * DPS
        step(i, lambda u: issue_some(1))

    issue_some(8)
    for g in range(G):
        for j in range(J):
            zo = jnp.where(diag, o_ref[g, 2 * j], o_ref[g, 2 * j + 1])
            oall_ref[j * R:(j + 1) * R, g * C:(g + 1) * C] = jnp.where(
                first_head, zo, pltpu.roll(zo, Sq, 0))

    pieces = []
    for k in range(NPIECE):
        last = min((k + 1) * PCH, NNORM)
        for par in (HI, LO):
            pieces.append((par * NPIECE + k, par * HALF + k * PCH * WOC,
                           (last - k * PCH) * WOC, par, last))
    for k in range(NSU):
        pieces.append((2 * NPIECE + k, 2 * HALF + k * UNIT, UNIT, LO,
                       NNORM + (k + 1) * UNIT // WOS))
    acc = None
    for p, r0, rn, par, last in pieces:
        issue_some(6)
        assert nxt[par] >= N * DPS + last
        lhs = oall_ref[:, r0:r0 + rn].astype(jnp.bfloat16)
        wait_all(wobuf.at[pl.ds(r0, rn)], osem.at[p])
        part = jnp.dot(lhs, wobuf[r0:r0 + rn, :], preferred_element_type=jnp.float32)
        acc = part if acc is None else acc + part
    for b in range(B):
        out_ref[b] = acc[b * Sq:(b + 1) * Sq, :].astype(out_ref.dtype)


def _compiler_params():
    params = dict(vmem_limit_bytes=64 * 1024 * 1024)
    if any(f.name == "disable_semaphore_checks"
           for f in dataclasses.fields(pltpu.CompilerParams)):
        params["disable_semaphore_checks"] = True
    return pltpu.CompilerParams(**params)


@jax.jit
def pallas_standalone__sliding_block_cached__sampling_kernel(
    x: jax.Array,
    k_cache: jax.Array,
    v_cache: jax.Array,
    wq: jax.Array,
    wo: jax.Array,
):
    B, Sq, D = x.shape
    Hq, Dh = 32, 192
    Hkv, Sk = k_cache.shape[1], k_cache.shape[2]
    W = min(4096, max(256, Sk // 4))
    assert Hq == Hkv and B % 2 == 0 and 2 * Sq == 8 and (Sk - W) % 128 == 0
    kt = jnp.swapaxes(k_cache, 2, 3).reshape(B * Hkv * Dh // 16, 2, 8, Sk)
    vt = jnp.swapaxes(v_cache, 2, 3).reshape(B * Hkv * Dh // 16, 2, 8, Sk)
    C = 2 * Dh
    G, R = Hq // 2, 2 * Sq
    _, _, npiece, nsu = _wo_plan(Hq * Dh)
    kern = functools.partial(_kernel, B=B, Sq=Sq, D=D, H=Hq, Dh=Dh, Sk=Sk, W=W,
                             scale=Dh ** -0.5)
    return pl.pallas_call(
        kern,
        in_specs=[pl.BlockSpec(memory_space=pl.ANY)] * 5,
        out_specs=pl.BlockSpec((B, Sq, D), lambda: (0, 0, 0)),
        out_shape=jax.ShapeDtypeStruct((B, Sq, D), x.dtype),
        scratch_shapes=[
            pltpu.VMEM((B, Sq, D), x.dtype),
            pltpu.VMEM((D, Hq * Dh), wq.dtype),
            pltpu.VMEM((Hq * Dh, D), wo.dtype),
            pltpu.VMEM((DIST + 1, 2, C // 16, 2, 8, W), k_cache.dtype),
            pltpu.VMEM((B * Sq, D), jnp.float32),
            pltpu.VMEM((B, G, R, C), jnp.float32),
            pltpu.VMEM((G, B, R, C), jnp.float32),
            pltpu.VMEM((B * Sq, Hq * Dh), jnp.float32),
            pltpu.SemaphoreType.DMA((2,)),
            pltpu.SemaphoreType.DMA((2 * npiece + nsu,)),
            pltpu.SemaphoreType.DMA((DIST + 1,)),
        ],
        compiler_params=_compiler_params(),
    )(x, wq, kt, vt, wo)
```
